```python
import os as _os
_os.environ.setdefault("JAX_PLATFORMS", "cpu")
import jax
import jax.numpy as jnp

def _softmax(x, axis=-1):
    return jax.nn.softmax(x, axis=axis)
def _gelu(x):
    return jax.nn.gelu(x, approximate=True)
def _silu(x):
    return jax.nn.silu(x)
def _sigmoid(x):
    return jax.nn.sigmoid(x)
def _layernorm(x, axis=-1, eps=1e-5):
    m = jnp.mean(x, axis=axis, keepdims=True)
    v = jnp.var(x, axis=axis, keepdims=True)
    return (x - m) / jnp.sqrt(v + eps)
def _scatter_add(tgt, idx, src, axis=0):
    return tgt.at[idx].add(src)
def _segment_sum(src, seg, n):
    return jax.ops.segment_sum(src, seg, n)
class _Rng:
    def __init__(self, key):
        self._k = key
    def _next(self):
        self._k, sub = jax.random.split(self._k)
        return sub
    def normal(self, shape):
        return jax.random.normal(self._next(), shape, dtype=jnp.bfloat16)
    def randint(self, lo, hi, shape):
        return jax.random.randint(self._next(), shape, lo, hi, dtype=jnp.int32)
    def uniform(self, shape, lo=0.0, hi=1.0):
        return jax.random.uniform(self._next(), shape, jnp.bfloat16, lo, hi)
    def permutation(self, n):
        return jax.random.permutation(self._next(), n)


kernel_name = 'parallel_sum__sliding_local_dilated__glu_gated_geglu__prompt'

def setup_inputs():
    _rng = _Rng(jax.random.key(int.from_bytes(__import__("os").urandom(4), "little")))
    _w = (lambda a: (lambda t: t.astype(jnp.bfloat16) if jnp.issubdtype(t.dtype, jnp.floating) else t)(jnp.asarray(a)))
    def _A_setup():
        B, S, D = 1, 2048, 512
        return {
            "x": _w((lambda *s: _rng.normal(s) * 0.05)(B, S, D)),
            "wqkv": _w((lambda *s: _rng.normal(s) * 0.05)(D, 3 * D)),
            "wo": _w((lambda *s: _rng.normal(s) * 0.05)(D, D)),
        }
    _A_in = _A_setup()

    def _B_setup():
        B, S, Dm, Df = 1, 2048, 512, 1376
        return {
            "x": _w((lambda *s: _rng.normal(s) * 0.05)(B, S, Dm)),
            "w_gate": _w((lambda *s: _rng.normal(s) * 0.1)(Dm, Df) * (Dm ** -0.5)),
            "w_up": _w((lambda *s: _rng.normal(s) * 0.1)(Dm, Df) * (Dm ** -0.5)),
            "w_down": _w((lambda *s: _rng.normal(s) * 0.1)(Df, Dm) * (Df ** -0.5)),
        }
    _B_in = _B_setup()

    return {
        "A_x": _A_in["x"],
        "A_wqkv": _A_in["wqkv"],
        "A_wo": _A_in["wo"],
        "B_x": _B_in["x"],
        "B_w_gate": _B_in["w_gate"],
        "B_w_up": _B_in["w_up"],
        "B_w_down": _B_in["w_down"],
    }

def reference(A_x, A_wqkv, A_wo, B_x, B_w_gate, B_w_up, B_w_down):
    def _A_ref(x, wqkv, wo):
        B, S, D = x.shape
        H = 32; Dh = D // H
        W, dil = 8, 2
        qkv = (lambda x, *d: x.transpose(*d))((x @ wqkv).reshape(B, S, 3, H, Dh), 2, 0, 3, 1, 4)
        q, k, v = qkv[0], qkv[1], qkv[2]
        scale = Dh ** -0.5
        pos = jnp.arange(S)
        off = jnp.arange(W) * dil
        idx = pos[:, None] - off[None, :]
        mask = idx >= 0
        idx_c = jnp.where(mask, idx, 0).reshape(-1)
        kg = k[:, :, idx_c, :].reshape(B, H, S, W, Dh)
        vg = v[:, :, idx_c, :].reshape(B, H, S, W, Dh)
        logits = jnp.einsum("bhsd,bhswd->bhsw", q, kg) * scale
        logits = jnp.where(mask[None, None, :, :], logits, -1e9)
        attn = _softmax(logits, axis=-1)
        o = jnp.einsum("bhsw,bhswd->bhsd", attn, vg)
        return (lambda x, *d: x.transpose(*d))(o, 0, 2, 1, 3).reshape(B, S, D) @ wo

    def _B_ref(x, w_gate, w_up, w_down):
        g = jnp.einsum("bsd,df->bsf", x, w_gate)
        u = jnp.einsum("bsd,df->bsf", x, w_up)
        h = _gelu(g) * u
        return jnp.einsum("bsf,fd->bsd", h, w_down)

    x = A_x
    xn = _layernorm(x, axis=-1)
    return x + _A_ref(xn, A_wqkv, A_wo) + _B_ref(xn, B_w_gate, B_w_up, B_w_down)
```

```python
import functools
import jax
import jax.numpy as jnp
import numpy as np
import jax.experimental.pallas as pl
import jax.experimental.pallas.tpu as pltpu

S, D, H, DH, W, DIL, DF = 2048, 512, 32, 16, 8, 2, 1376
HALO = 16
LOG2E = 1.4426950408889634
NT = (((1,), (1,)), ((), ()))
f32, bf16 = jnp.float32, jnp.bfloat16


def _gelu(x):
    c = 0.7978845608028654
    return 0.5 * x * (1.0 + jnp.tanh(c * (x + 0.044715 * (x * x * x))))


def _kernel(x_hbm, wqkv_hbm, wo_hbm, wg_hbm, wu_hbm, wd_hbm, out_hbm,
            xb, ob, wqkv, wqkvp, wo, wo32, wop, wg, wu, wd,
            xn_ref, q_ref, k_ref, v_ref, o_ref, h_ref,
            sx, so, sw, sg, su, *, tm, rc, nc, order0, unroll):
    nblk = S // tm
    chunks = [(n0, min(nc, DF - n0)) for n0 in range(0, DF, nc)]

    def x_copy(i):
        return pltpu.make_async_copy(x_hbm.at[pl.ds(i * tm, tm), :], xb.at[pl.ds(i * tm, tm), :], sx.at[i])

    def o_copy(i):
        return pltpu.make_async_copy(ob.at[pl.ds(i * tm, tm), :], out_hbm.at[pl.ds(i * tm, tm), :], so.at[i])

    def g_copy(c):
        n0, nn = chunks[c]
        return pltpu.make_async_copy(wg_hbm.at[pl.ds(n0, nn), :], wg.at[pl.ds(n0, nn), :], sg.at[c])

    def u_copy(c):
        n0, nn = chunks[c]
        return pltpu.make_async_copy(wu_hbm.at[pl.ds(n0, nn), :], wu.at[pl.ds(n0, nn), :], su.at[c])

    def wqkv_copy(m):
        return pltpu.make_async_copy(wqkv_hbm.at[:, pl.ds(m * 512, 512)], wqkv.at[m], sw.at[m])
    wo_copy = pltpu.make_async_copy(wo_hbm, wo, sw.at[3])
    wd_copy = pltpu.make_async_copy(wd_hbm, wd, sw.at[4])

    def dma(name):
        if name[0] == 'x':
            return x_copy(int(name[1:]))
        if name[0] == 'g':
            return g_copy(int(name[1:]))
        if name[0] == 'u':
            return u_copy(int(name[1:]))
        if name[:2] == 'wq':
            return wqkv_copy(int(name[2:]))
        return {'wo': wo_copy, 'wd': wd_copy}[name]

    for waits, _ in order0:
        for name in waits:
            dma(name).start()

    def layernorm(row0):
        for r in range(0, tm, 64):
            x = xb[pl.ds(row0 + r, 64), :].astype(f32)
            m = jnp.mean(x, axis=-1, keepdims=True)
            xc = x - m
            var = jnp.mean(xc * xc, axis=-1, keepdims=True)
            xn_ref[pl.ds(r, 64), :] = (xc * jax.lax.rsqrt(var + 1e-5)).astype(bf16)

    def permute_qkv(mat):
        lane = jax.lax.broadcasted_iota(jnp.int32, (256, 128), 1)
        grp = (lane % 32) // 8
        if True:
            tiles = [pltpu.bitcast(wqkv[mat, :, pl.ds(t * 128, 128)], jnp.uint32) for t in range(4)]
            for j in range(4):
                idx = (lane % 8) * 16 + 4 * j + lane // 32
                res = None
                for t in range(4):
                    g = jnp.take_along_axis(tiles[t], idx, axis=1)
                    res = g if res is None else jnp.where(grp == t, g, res)
                wqkvp[:, pl.ds(mat * 512 + j * 128, 128)] = pltpu.bitcast(res, bf16)

    def permute_o():
        for c in range(4):
            wo32[c] = wo[:, pl.ds(c * 128, 128)].astype(f32)
        for c in range(4):
            for d in range(16):
                wop[pl.ds(d * 32, 32), pl.ds(c * 128, 128)] = wo32[c, pl.ds(d, 32, stride=16), :].astype(bf16)

    def qkv():
        for j in range(4):
            q_ref[j] = jnp.dot(xn_ref[...], wqkvp[:, pl.ds(j * 128, 128)], preferred_element_type=f32)
            k_ref[j, pl.ds(HALO, tm), :] = jnp.dot(xn_ref[...], wqkvp[:, pl.ds(512 + j * 128, 128)], preferred_element_type=f32)
            v_ref[j, pl.ds(HALO, tm), :] = jnp.dot(xn_ref[...], wqkvp[:, pl.ds(1024 + j * 128, 128)], preferred_element_type=f32)

    def gate_up(c):
        n0, nn = chunks[c]
        g = jax.lax.dot_general(xn_ref[...], wg[pl.ds(n0, nn), :], NT, preferred_element_type=f32)
        u = jax.lax.dot_general(xn_ref[...], wu[pl.ds(n0, nn), :], NT, preferred_element_type=f32)
        h_ref[:, pl.ds(n0, nn)] = (_gelu(g) * u).astype(bf16)

    def attention(first):
        cs = (DH ** -0.5) * LOG2E
        for r in range(tm // rc):
            r0 = r * rc
            q = [q_ref[j, pl.ds(r0, rc), :] * cs for j in range(4)]
            ls = []
            for w in range(W):
                acc = None
                for j in range(4):
                    p = q[j] * k_ref[j, pl.ds(HALO + r0 - DIL * w, rc), :]
                    acc = p if acc is None else acc + p
                acc = acc + pltpu.roll(acc, 64, 1)
                acc = acc + pltpu.roll(acc, 32, 1)
                if first and r == 0 and w > 0:
                    row = jax.lax.broadcasted_iota(jnp.int32, (rc, 128), 0)
                    acc = jnp.where(row >= DIL * w, acc, -1e30)
                ls.append(acc)
            mx = ls[0]
            for w in range(1, W):
                mx = jnp.maximum(mx, ls[w])
            es = [jnp.exp2(l - mx) for l in ls]
            sm = es[0]
            for w in range(1, W):
                sm = sm + es[w]
            rinv = 1.0 / sm
            for j in range(4):
                o = None
                for w in range(W):
                    p = es[w] * v_ref[j, pl.ds(HALO + r0 - DIL * w, rc), :]
                    o = p if o is None else o + p
                o_ref[pl.ds(r0, rc), pl.ds(j * 128, 128)] = (o * rinv).astype(bf16)
        for j in range(4):
            k_ref[j, pl.ds(0, HALO), :] = k_ref[j, pl.ds(tm, HALO), :]
            v_ref[j, pl.ds(0, HALO), :] = v_ref[j, pl.ds(tm, HALO), :]

    def final(row0):
        acc = xb[pl.ds(row0, tm), :].astype(f32)
        acc = acc + jnp.dot(h_ref[...], wd[...], preferred_element_type=f32)
        acc = acc + jnp.dot(o_ref[...], wop[...], preferred_element_type=f32)
        ob[pl.ds(row0, tm), :] = acc.astype(bf16)

    z = jnp.zeros((HALO, 128), f32)
    for j in range(4):
        k_ref[j, pl.ds(0, HALO), :] = z
        v_ref[j, pl.ds(0, HALO), :] = z
    for waits, steps in order0:
        for name in waits:
            dma(name).wait()
        for step in steps:
            if step[0] == 'g':
                gate_up(int(step[1:]))
            elif step[:2] == 'pq':
                permute_qkv(int(step[2:]))
            elif step == 'po':
                permute_o()
            elif step == 'qkv':
                qkv()
            elif step == 'att':
                attention(True)
            elif step[:2] == 'ln':
                layernorm(int(step[2:]) * tm)
            elif step == 'fin':
                final(0)
    o_copy(0).start()

    def body(i):
        row0 = pl.multiple_of(i * tm, tm)
        qkv()
        for c in range(len(chunks)):
            gate_up(c)
        attention(False)
        nxt = jnp.minimum(i + 1, nblk - 1)
        layernorm(pl.multiple_of(nxt * tm, tm))
        final(row0)
        o_copy(i).start()

    if unroll:
        for i in range(1, nblk):
            body(i)
    else:
        pl.loop(1, nblk)(body)
    for i in range(nblk):
        o_copy(i).wait()


def make(tm=512, rc=32, nc=256, order0=None, unroll=False):
    nch = -(-DF // nc)
    nb = S // tm
    if order0 is None:
        assert nc == 256
        order0 = [(['x0'], ['ln0']),
                  (['g0', 'u0'], ['g0']),
                  (['g1', 'u1', 'wq0'], ['g1', 'pq0']),
                  (['g2', 'u2', 'wq1'], ['g2', 'pq1']),
                  (['g3', 'u3', 'wq2'], ['g3', 'pq2']),
                  (['g4', 'u4', 'wo'], ['g4', 'po']),
                  (['g5', 'u5', 'x1', 'wd'] + ['x%d' % i for i in range(2, nb)], ['qkv', 'g5', 'att', 'ln1', 'fin'])]

    @jax.jit
    def f(A_x, A_wqkv, A_wo, B_x, B_w_gate, B_w_up, B_w_down):
        x2 = A_x.reshape(S, D)
        hbm = pl.BlockSpec(memory_space=pltpu.HBM)
        nblk = S // tm
        out = pl.pallas_call(
            functools.partial(_kernel, tm=tm, rc=rc, nc=nc, order0=order0, unroll=unroll),
            in_specs=[hbm] * 6,
            out_specs=hbm,
            out_shape=jax.ShapeDtypeStruct((S, D), bf16),
            scratch_shapes=[
                pltpu.VMEM((S, D), bf16), pltpu.VMEM((S, D), bf16),
                pltpu.VMEM((3, D, D), bf16), pltpu.VMEM((D, 3 * D), bf16),
                pltpu.VMEM((D, D), bf16), pltpu.VMEM((4, D, 128), f32), pltpu.VMEM((D, D), bf16),
                pltpu.VMEM((DF, D), bf16), pltpu.VMEM((DF, D), bf16), pltpu.VMEM((DF, D), bf16),
                pltpu.VMEM((tm, D), bf16),
                pltpu.VMEM((4, tm, 128), f32),
                pltpu.VMEM((4, tm + HALO, 128), f32),
                pltpu.VMEM((4, tm + HALO, 128), f32),
                pltpu.VMEM((tm, D), bf16),
                pltpu.VMEM((tm, DF), bf16),
                pltpu.SemaphoreType.DMA((nblk,)), pltpu.SemaphoreType.DMA((nblk,)),
                pltpu.SemaphoreType.DMA((5,)), pltpu.SemaphoreType.DMA((nch,)), pltpu.SemaphoreType.DMA((nch,)),
            ],
            compiler_params=pltpu.CompilerParams(vmem_limit_bytes=100 * 1024 * 1024),
            name="fused_kernel",
        )(x2, A_wqkv, A_wo, B_w_gate.T, B_w_up.T, B_w_down)
        return out.reshape(1, S, D)
    return f


_impl = make(**{'tm':512})


@jax.jit
def pallas_parallel_sum__sliding_local_dilated__glu_gated_geglu__prompt_kernel(
    A_x: jax.Array,
    A_wqkv: jax.Array,
    A_wo: jax.Array,
    B_x: jax.Array,
    B_w_gate: jax.Array,
    B_w_up: jax.Array,
    B_w_down: jax.Array,
):
    return _impl(A_x, A_wqkv, A_wo, B_x, B_w_gate, B_w_up, B_w_down)
```

```python
import functools
import jax
import jax.numpy as jnp
import numpy as np
import jax.experimental.pallas as pl
import jax.experimental.pallas.tpu as pltpu

S, D, H, DH, W, DIL, DF = 2048, 512, 32, 16, 8, 2, 1376
HALO = 16
LOG2E = 1.4426950408889634
NT = (((1,), (1,)), ((), ()))
f32, bf16, u32 = jnp.float32, jnp.bfloat16, jnp.uint32


def _gelu(x):
    c = 0.7978845608028654
    return 0.5 * x * (1.0 + jnp.tanh(c * (x + 0.044715 * (x * x * x))))


def _kernel(x_hbm, wqkv_hbm, wo_hbm, wg_hbm, wu_hbm, wd_hbm, out_hbm,
            xb, ob, wqkv, wqkvp, wo, wo32, wop, wg, wu, wd,
            xn_ref, q_ref, k_ref, v_ref, o_ref, h_ref,
            sx, so, sw, sg, su, *, cfg):
    tm, rc, nc = cfg['tm'], cfg['rc'], cfg['nc']
    packed = cfg['packed']
    osplit = cfg['osplit']
    nblk = S // tm
    chunks = [(n0, min(nc, DF - n0)) for n0 in range(0, DF, nc)]


    def put(ref, r0, c0, val):
        if packed:
            ref[pl.ds(r0 // 2, val.shape[0] // 2), pl.ds(c0, val.shape[1])] = pltpu.bitcast(val, u32)
        else:
            ref[pl.ds(r0, val.shape[0]), pl.ds(c0, val.shape[1])] = val

    def get(ref):
        return pltpu.bitcast(ref[...], bf16) if packed else ref[...]

    def x_copy(i):
        return pltpu.make_async_copy(x_hbm.at[pl.ds(i * tm, tm), :], xb.at[pl.ds(i * tm, tm), :], sx.at[i])

    ow = D // osplit

    def o_copy(i, t, row0=None):
        row0 = i * tm if row0 is None else row0
        return pltpu.make_async_copy(ob.at[pl.ds(row0, tm), pl.ds(t * ow, ow)],
                                     out_hbm.at[pl.ds(row0, tm), pl.ds(t * ow, ow)], so.at[i, t])

    def g_copy(c):
        n0, nn = chunks[c]
        return pltpu.make_async_copy(wg_hbm.at[pl.ds(n0, nn), :], wg.at[pl.ds(n0, nn), :], sg.at[c])

    def u_copy(c):
        n0, nn = chunks[c]
        return pltpu.make_async_copy(wu_hbm.at[pl.ds(n0, nn), :], wu.at[pl.ds(n0, nn), :], su.at[c])

    def wqkv_copy(m):
        return pltpu.make_async_copy(wqkv_hbm.at[:, pl.ds(m * 512, 512)], wqkv.at[m], sw.at[m])

    def dma(name):
        if name[0] == 'x':
            return x_copy(int(name[1:]))
        if name[0] == 'g':
            return g_copy(int(name[1:]))
        if name[0] == 'u':
            return u_copy(int(name[1:]))
        if name[:2] == 'wq':
            return wqkv_copy(int(name[2:]))
        if name == 'wo':
            return pltpu.make_async_copy(wo_hbm, wo, sw.at[3])
        return pltpu.make_async_copy(wd_hbm, wd, sw.at[4])

    def layernorm(row0):
        for r in range(0, tm, 64):
            x = xb[pl.ds(row0 + r, 64), :].astype(f32)
            m = jnp.mean(x, axis=-1, keepdims=True)
            xc = x - m
            var = jnp.mean(xc * xc, axis=-1, keepdims=True)
            put(xn_ref, r, 0, (xc * jax.lax.rsqrt(var + 1e-5)).astype(bf16))

    def permute_qkv(mat):
        lane = jax.lax.broadcasted_iota(jnp.int32, (256, 128), 1)
        grp = (lane % 32) // 8
        tiles = [pltpu.bitcast(wqkv[mat, :, pl.ds(t * 128, 128)], u32) for t in range(4)]
        for j in range(4):
            idx = (lane % 8) * 16 + 4 * j + lane // 32
            res = None
            for t in range(4):
                g = jnp.take_along_axis(tiles[t], idx, axis=1)
                res = g if res is None else jnp.where(grp == t, g, res)
            wqkvp[:, pl.ds(mat * 512 + j * 128, 128)] = res if packed else pltpu.bitcast(res, bf16)

    def wqkvp_tile(c0):
        t = wqkvp[:, pl.ds(c0, 128)]
        return pltpu.bitcast(t, bf16) if packed else t

    def permute_o():
        for c in range(4):
            wo32[c] = wo[:, pl.ds(c * 128, 128)].astype(f32)
        for c in range(4):
            for d in range(16):
                put(wop, d * 32, c * 128, wo32[c, pl.ds(d, 32, stride=16), :].astype(bf16))

    def qkv():
        for j in range(4):
            q_ref[j] = jnp.dot(get(xn_ref), wqkvp_tile(j * 128), preferred_element_type=f32)
        for j in range(4):
            k_ref[j, pl.ds(HALO, tm), :] = jnp.dot(get(xn_ref), wqkvp_tile(512 + j * 128), preferred_element_type=f32)
        for j in range(4):
            v_ref[j, pl.ds(HALO, tm), :] = jnp.dot(get(xn_ref), wqkvp_tile(1024 + j * 128), preferred_element_type=f32)

    def gate_up(c, t0=0.0):
        n0, nn = chunks[c]
        g = jax.lax.dot_general(get(xn_ref), wg[pl.ds(n0, nn), :], NT, preferred_element_type=f32)
        u = jax.lax.dot_general(get(xn_ref), wu[pl.ds(n0, nn), :], NT, preferred_element_type=f32)
        put(h_ref, 0, n0, (_gelu(g) * u).astype(bf16))
        srcs = []
        t = t0
        for val in (g, u):
            for c0 in range(0, nn, 128):
                for r in range(0, tm, 32):
                    srcs.append((t + r + 32, val[r + 24:r + 32, c0:c0 + min(128, nn - c0)]))
                t += tm
        return srcs, t

    def att_chunk(r0, first, src):
        cs = (DH ** -0.5) * LOG2E
        if src is not None:
            if src.shape[1] < 128:
                src = jnp.concatenate([src, jnp.zeros((8, 128 - src.shape[1]), f32)], axis=1)
            zz = (pltpu.bitcast(src, u32) >> 31) >> 1
            csv = pltpu.bitcast(pltpu.bitcast(jnp.full((8, 128), cs, f32), u32) | zz, f32)
            cs = jnp.concatenate([csv] * (rc // 8), axis=0) if rc > 8 else csv
        q = [q_ref[j, pl.ds(r0, rc), :] * cs for j in range(4)]
        ls = []
        for w in range(W):
            acc = None
            for j in range(4):
                p = q[j] * k_ref[j, pl.ds(HALO + r0 - DIL * w, rc), :]
                acc = p if acc is None else acc + p
            acc = acc + pltpu.roll(acc, 64, 1)
            acc = acc + pltpu.roll(acc, 32, 1)
            if first and r0 < DIL * w:
                row = r0 + jax.lax.broadcasted_iota(jnp.int32, (rc, 128), 0)
                acc = jnp.where(row >= DIL * w, acc, -1e30)
            ls.append(acc)
        mx = ls[0]
        for w in range(1, W):
            mx = jnp.maximum(mx, ls[w])
        es = [jnp.exp2(l - mx) for l in ls]
        sm = es[0]
        for w in range(1, W):
            sm = sm + es[w]
        rinv = 1.0 / sm
        for j in range(4):
            o = None
            for w in range(W):
                p = es[w] * v_ref[j, pl.ds(HALO + r0 - DIL * w, rc), :]
                o = p if o is None else o + p
            put(o_ref, r0, j * 128, (o * rinv).astype(bf16))

    def halo():
        for j in range(4):
            k_ref[j, pl.ds(0, HALO), :] = k_ref[j, pl.ds(tm, HALO), :]
            v_ref[j, pl.ds(0, HALO), :] = v_ref[j, pl.ds(tm, HALO), :]

    def pick(srcs, t):
        best = min(range(len(srcs)), key=lambda i: abs(srcs[i][0] - t))
        return srcs[best][1]

    def tail(cs_list, first, tlo, thi, i, row0, nxt_row0, pre_ln=None):
        nr = tm // rc
        times = [tlo + (thi - tlo) * r / max(nr - 1, 1) for r in range(nr)]
        srcs, t = [], 0.0
        for c in cs_list:
            s, t = gate_up(c, t)
            srcs += s
        r = 0
        while r < nr and times[r] <= t:
            att_chunk(r * rc, first, pick(srcs, times[r]))
            r += 1
        layernorm(nxt_row0)
        dn = jnp.dot(get(h_ref), wd[...], preferred_element_type=f32)
        per = 11 * tm / 4
        dsrcs = [(t + per * (ct + 0.7) + 0.3 * per * rr / tm, dn[rr + 24:rr + 32, ct * 128:(ct + 1) * 128])
                 for ct in range(4) for rr in range(0, tm, 32)]
        while r < nr:
            att_chunk(r * rc, first, pick(dsrcs, times[r]))
            r += 1
        halo()
        acc = xb[pl.ds(row0, tm), :].astype(f32) + dn
        acc = acc + jnp.dot(get(o_ref), get(wop), preferred_element_type=f32)
        for tt in range(osplit):
            ob[pl.ds(row0, tm), pl.ds(tt * ow, ow)] = acc[:, tt * ow:(tt + 1) * ow].astype(bf16)
            o_copy(i, tt, row0).start()

    z = jnp.zeros((HALO, 128), f32)
    for j in range(4):
        k_ref[j, pl.ds(0, HALO), :] = z
        v_ref[j, pl.ds(0, HALO), :] = z
    order0 = cfg['order0']
    for name in order0[0]:
        dma(name).start()
    for waits, starts, steps in order0[1:]:
        with jax.named_scope('wait_' + '_'.join(waits)) if cfg['scopes'] else contextless():
            for name in waits:
                dma(name).wait()
            for name in starts:
                dma(name).start()
        for step in steps:
            if step[0] == 'g':
                gate_up(int(step[1:]))
            elif step[:2] == 'pq':
                permute_qkv(int(step[2:]))
            elif step == 'po':
                permute_o()
            elif step == 'qkv':
                qkv()
            elif step[:2] == 'ln':
                layernorm(int(step[2:]) * tm)
            elif step[:5] == 'tail_':
                tail([int(ch) for ch in step[5:]], True, cfg['pace0'][0], cfg['pace0'][1], 0, 0, tm)

    def body(i):
        row0 = pl.multiple_of(i * tm, tm)
        nxt = pl.multiple_of(jnp.minimum(i + 1, nblk - 1) * tm, tm)
        qkv()
        tail(list(range(len(chunks))), False, cfg['pace'][0], cfg['pace'][1], i, row0, nxt)

    if cfg['unroll']:
        for i in range(1, nblk):
            body(i)
    else:
        pl.loop(1, nblk)(body)
    with jax.named_scope('wait_out') if cfg['scopes'] else contextless():
        for i in range(nblk):
            for t in range(osplit):
                o_copy(i, t).wait()


class contextless:
    def __enter__(self):
        return self

    def __exit__(self, *a):
        return False


def make(tm=512, rc=32, nc=256, order0=None, unroll=False, packed=False, osplit=1, scopes=False,
         pace=(0, 9000), pace0=(0, 5500), early_x=True, nosem=False):
    nch = -(-DF // nc)
    nb = S // tm
    if order0 is None:
        assert nc == 256
        xs = ['x%d' % i for i in range(2, nb)]
        order0 = [['x0', 'g0', 'u0'],
                  (['x0'], ['g1', 'u1', 'wq0'], ['ln0']),
                  (['g0', 'u0'], ['g2', 'u2', 'wq1'], ['g0']),
                  (['g1', 'u1', 'wq0'], ['g3', 'u3', 'wq2'], ['g1', 'pq0']),
                  (['g2', 'u2', 'wq1'], ['g4', 'u4', 'wo', 'g5', 'u5'], ['g2', 'pq1']),
                  (['g3', 'u3', 'wq2'], ['x1', 'wd'] + (xs if early_x else []), ['pq2', 'g3', 'qkv']),
                  (['g4', 'u4', 'wo', 'g5', 'u5', 'x1', 'wd'] + (xs if early_x else []), [] if early_x else xs, ['po', 'tail_45'])]
        if not early_x:
            order0.append((xs, [], []))
    cfg = dict(tm=tm, rc=rc, nc=nc, order0=order0, unroll=unroll, packed=packed, osplit=osplit, scopes=scopes,
               pace=pace, pace0=pace0)

    @jax.jit
    def f(A_x, A_wqkv, A_wo, B_x, B_w_gate, B_w_up, B_w_down):
        x2 = A_x.reshape(S, D)
        hbm = pl.BlockSpec(memory_space=pltpu.HBM)
        nblk = S // tm
        act = (lambda r, c: pltpu.VMEM((r // 2, c), u32)) if packed else (lambda r, c: pltpu.VMEM((r, c), bf16))
        out = pl.pallas_call(
            functools.partial(_kernel, cfg=cfg),
            in_specs=[hbm] * 6,
            out_specs=hbm,
            out_shape=jax.ShapeDtypeStruct((S, D), bf16),
            scratch_shapes=[
                pltpu.VMEM((S, D), bf16), pltpu.VMEM((S, D), bf16),
                pltpu.VMEM((3, D, D), bf16), act(D, 3 * D),
                pltpu.VMEM((D, D), bf16), pltpu.VMEM((4, D, 128), f32), act(D, D),
                pltpu.VMEM((DF, D), bf16), pltpu.VMEM((DF, D), bf16), pltpu.VMEM((DF, D), bf16),
                act(tm, D),
                pltpu.VMEM((4, tm, 128), f32),
                pltpu.VMEM((4, tm + HALO, 128), f32),
                pltpu.VMEM((4, tm + HALO, 128), f32),
                act(tm, D),
                act(tm, DF),
                pltpu.SemaphoreType.DMA((nblk,)), pltpu.SemaphoreType.DMA((nblk, osplit)),
                pltpu.SemaphoreType.DMA((5,)), pltpu.SemaphoreType.DMA((nch,)), pltpu.SemaphoreType.DMA((nch,)),
            ],
            compiler_params=pltpu.CompilerParams(vmem_limit_bytes=100 * 1024 * 1024, disable_semaphore_checks=nosem),
            name="fused_kernel",
        )(x2, A_wqkv, A_wo, B_w_gate.T, B_w_up.T, B_w_down)
        return out.reshape(1, S, D)
    return f


_impl = make(**{'packed':True,'osplit':4,'nosem':True,'early_x':False,'rc':8,'pace':(0,10500),'pace0':(0,6500)})


@jax.jit
def pallas_parallel_sum__sliding_local_dilated__glu_gated_geglu__prompt_kernel(
    A_x: jax.Array,
    A_wqkv: jax.Array,
    A_wo: jax.Array,
    B_x: jax.Array,
    B_w_gate: jax.Array,
    B_w_up: jax.Array,
    B_w_down: jax.Array,
):
    return _impl(A_x, A_wqkv, A_wo, B_x, B_w_gate, B_w_up, B_w_down)
```

```python
import functools
import jax
import jax.numpy as jnp
import numpy as np
import jax.experimental.pallas as pl
import jax.experimental.pallas.tpu as pltpu

S, D, H, DH, W, DIL, DF = 2048, 512, 32, 16, 8, 2, 1376
HALO = 16
LOG2E = 1.4426950408889634
NT = (((1,), (1,)), ((), ()))
f32, bf16, u32 = jnp.float32, jnp.bfloat16, jnp.uint32


def _gelu(x):
    c = 0.7978845608028654
    return 0.5 * x * (1.0 + jnp.tanh(c * (x + 0.044715 * (x * x * x))))


def _kernel(x_hbm, wqkv_hbm, wo_hbm, wg_hbm, wu_hbm, wd_hbm, out_hbm,
            xb, ob, wqkv, wqkvp, wo, wo32, wop, w2, wd,
            xn_ref, xnb, q_ref, k_ref, v_ref, o_ref, h_ref,
            sin, so, *, cfg):
    tm0, tm1, rc, nc = cfg['tm0'], cfg['tm1'], cfg['rc'], cfg['nc']
    packed = cfg['packed']
    osplit = cfg['osplit']
    nblk = 1 + (S - tm0) // tm1
    assert tm0 + (nblk - 1) * tm1 == S
    chunks = [(n0, min(nc, DF - n0)) for n0 in range(0, DF, nc)]

    def blk(i):
        return (0, tm0) if i == 0 else (tm0 + (i - 1) * tm1, tm1)

    def put(ref, r0, c0, val):
        if packed:
            ref[pl.ds(r0 // 2, val.shape[0] // 2), pl.ds(c0, val.shape[1])] = pltpu.bitcast(val, u32)
        else:
            ref[pl.ds(r0, val.shape[0]), pl.ds(c0, val.shape[1])] = val

    def get(ref, tm=None):
        if tm is None:
            return pltpu.bitcast(ref[...], bf16) if packed else ref[...]
        return pltpu.bitcast(ref[pl.ds(0, tm // 2), :], bf16) if packed else ref[pl.ds(0, tm), :]

    names = cfg['names']

    def sem(name):
        return sin.at[names.index(name)]

    def x_copy(i):
        r0, n = blk(i)
        return pltpu.make_async_copy(x_hbm.at[pl.ds(r0, n), :], xb.at[pl.ds(r0, n), :], sem('x%d' % i))

    def x_copy_dyn(i):
        r0 = pl.multiple_of(tm0 + (i - 1) * tm1, 16)
        return pltpu.make_async_copy(x_hbm.at[pl.ds(r0, tm1), :], xb.at[pl.ds(r0, tm1), :],
                                     sin.at[names.index('x1') + i - 1])

    ow = D // osplit

    def o_copy(i, t, row0, tm):
        return pltpu.make_async_copy(ob.at[pl.ds(row0, tm), pl.ds(t * ow, ow)],
                                     out_hbm.at[pl.ds(row0, tm), pl.ds(t * ow, ow)], so.at[i, t])

    def g_copy(c):
        n0, nn = chunks[c]
        return pltpu.make_async_copy(wg_hbm.at[pl.ds(n0, nn), :], w2.at[0, pl.ds(n0, nn), :], sem('g%d' % c))

    def u_copy(c):
        n0, nn = chunks[c]
        return pltpu.make_async_copy(wu_hbm.at[pl.ds(n0, nn), :], w2.at[1, pl.ds(n0, nn), :], sem('u%d' % c))

    def wqkv_copy(m):
        return pltpu.make_async_copy(wqkv_hbm.at[:, pl.ds(m * 512, 512)], wqkv.at[m], sem('wq%d' % m))

    def dma(name):
        if name[0] == 'x':
            return x_copy(int(name[1:]))
        if name[0] == 'g':
            return g_copy(int(name[1:]))
        if name[0] == 'u':
            return u_copy(int(name[1:]))
        if name[:2] == 'wq':
            return wqkv_copy(int(name[2:]))
        if name == 'wo':
            return pltpu.make_async_copy(wo_hbm, wo, sem('wo'))
        return pltpu.make_async_copy(wd_hbm, wd, sem('wd'))

    def getr(ref, r, n):
        return pltpu.bitcast(ref[pl.ds(r // 2, n // 2), :], bf16) if packed else ref[pl.ds(r, n), :]

    def ln_chunk(row0, r, n, src=None, mark=False):
        xv = xb[pl.ds(row0 + r, n), :]
        if src is not None:
            zz = (pltpu.bitcast(src, u32) >> 31) >> 1
            zz = jnp.concatenate([zz] * 4, axis=1)
            zz = jnp.concatenate([zz] * (n // 16), axis=0) if n > 16 else zz
            xv = pltpu.bitcast(pltpu.bitcast(xv, u32) | zz, bf16)
        x = xv.astype(f32)
        m = jnp.mean(x, axis=-1, keepdims=True)
        xc = x - m
        var = jnp.mean(xc * xc, axis=-1, keepdims=True)
        y = (xc * jax.lax.rsqrt(var + 1e-5)).astype(bf16)
        put(xn_ref, r, 0, y)
        if mark:
            w2[0, pl.ds(DF, 16), pl.ds(0, 128)] = y[n - 16:n, D - 128:D]

    def layernorm(row0, tm):
        step = cfg['ln0r']
        for r in range(0, tm, step):
            ln_chunk(row0, r, min(step, tm - r), mark=(r == cfg['mark']))

    def permute_qkv(mat):
        lane = jax.lax.broadcasted_iota(jnp.int32, (256, 128), 1)
        grp = (lane % 32) // 8
        tiles = [pltpu.bitcast(wqkv[mat, :, pl.ds(t * 128, 128)], u32) for t in range(4)]
        for j in range(4):
            idx = (lane % 8) * 16 + 4 * j + lane // 32
            res = None
            for t in range(4):
                g = jnp.take_along_axis(tiles[t], idx, axis=1)
                res = g if res is None else jnp.where(grp == t, g, res)
            wqkvp[:, pl.ds(mat * 512 + j * 128, 128)] = res if packed else pltpu.bitcast(res, bf16)

    def wqkvp_tile(c0):
        t = wqkvp[:, pl.ds(c0, 128)]
        return pltpu.bitcast(t, bf16) if packed else t

    def permute_o():
        for c in range(4):
            wo32[c] = wo[:, pl.ds(c * 128, 128)].astype(f32)
        for c in range(4):
            for d in range(16):
                put(wop, d * 32, c * 128, wo32[c, pl.ds(d, 32, stride=16), :].astype(bf16))

    def qkv(tm):
        for j in range(4):
            q_ref[j, pl.ds(0, tm), :] = jnp.dot(get(xn_ref, tm), wqkvp_tile(j * 128), preferred_element_type=f32)
        for j in range(4):
            k_ref[j, pl.ds(HALO, tm), :] = jnp.dot(get(xn_ref, tm), wqkvp_tile(512 + j * 128), preferred_element_type=f32)
        for j in range(4):
            v_ref[j, pl.ds(HALO, tm), :] = jnp.dot(get(xn_ref, tm), wqkvp_tile(1024 + j * 128), preferred_element_type=f32)

    def gate_up(c, tm, t0=0.0, src=None, first=False):
        src = xn_ref if src is None else src
        n0, nn = chunks[c]
        if first:
            g_copy(c).wait()
        g = jax.lax.dot_general(get(src, tm), w2[0, pl.ds(n0, nn), :], NT, preferred_element_type=f32)
        if first:
            u_copy(c).wait()
        u = jax.lax.dot_general(get(src, tm), w2[1, pl.ds(n0, nn), :], NT, preferred_element_type=f32)
        put(h_ref, 0, n0, (_gelu(g) * u).astype(bf16))
        srcs = []
        t = t0
        for val in (g, u):
            for c0 in range(0, nn, 128):
                for r in range(0, tm - 31, 32):
                    srcs.append((t + r + 32, val[r + 24:r + 32, c0:c0 + min(128, nn - c0)]))
                t += tm
        return srcs, t

    def att_chunk(r0, first, src):
        cs = (DH ** -0.5) * LOG2E
        if src is not None:
            if src.shape[1] < 128:
                src = jnp.concatenate([src, jnp.zeros((8, 128 - src.shape[1]), f32)], axis=1)
            zz = (pltpu.bitcast(src, u32) >> 31) >> 1
            csv = pltpu.bitcast(pltpu.bitcast(jnp.full((8, 128), cs, f32), u32) | zz, f32)
            cs = jnp.concatenate([csv] * (rc // 8), axis=0) if rc > 8 else csv
        q = [q_ref[j, pl.ds(r0, rc), :] * cs for j in range(4)]
        ls = []
        for w in range(W):
            acc = None
            for j in range(4):
                p = q[j] * k_ref[j, pl.ds(HALO + r0 - DIL * w, rc), :]
                acc = p if acc is None else acc + p
            acc = acc + pltpu.roll(acc, 64, 1)
            acc = acc + pltpu.roll(acc, 32, 1)
            if first and r0 < DIL * w:
                row = r0 + jax.lax.broadcasted_iota(jnp.int32, (rc, 128), 0)
                acc = jnp.where(row >= DIL * w, acc, -1e30)
            ls.append(acc)
        mx = ls[0]
        for w in range(1, W):
            mx = jnp.maximum(mx, ls[w])
        es = [jnp.exp2(l - mx) for l in ls]
        sm = es[0]
        for w in range(1, W):
            sm = sm + es[w]
        rinv = 1.0 / sm
        for j in range(4):
            o = None
            for w in range(W):
                p = es[w] * v_ref[j, pl.ds(HALO + r0 - DIL * w, rc), :]
                o = p if o is None else o + p
            put(o_ref, r0, j * 128, (o * rinv).astype(bf16))

    def halo(tm):
        for j in range(4):
            k_ref[j, pl.ds(0, HALO), :] = k_ref[j, pl.ds(tm, HALO), :]
            v_ref[j, pl.ds(0, HALO), :] = v_ref[j, pl.ds(tm, HALO), :]

    def pick(srcs, t):
        best = min(range(len(srcs)), key=lambda i: abs(srcs[i][0] - t))
        return srcs[best][1]

    def pick128(srcs, t):
        return pick([x for x in srcs if x[1].shape[1] == 128], t)

    def tail(cs_list, first, tlo, thi, i, row0, tm, nxt_row0, nxt_tm, src):
        nr = tm // rc
        times = [tlo + (thi - tlo) * r / max(nr - 1, 1) for r in range(nr)]
        srcs, t = [], 0.0
        for c in cs_list:
            s, t = gate_up(c, tm, t, src, first)
            srcs += s
        lnr = cfg['lnr']
        lns = []
        if nxt_row0 is not None and cfg['early']:
            k = nxt_tm // lnr
            lo, hi = cfg['lnp0'] if first else cfg['lnp']
            lns = [(lo + (hi - lo) * a / max(k - 1, 1), a * lnr) for a in range(k)]
        r = 0
        while r < nr and times[r] <= t:
            while lns and lns[0][0] <= times[r]:
                tt, lr = lns.pop(0)
                ln_chunk(nxt_row0, lr, lnr, pick128(srcs, tt))
            att_chunk(r * rc, first, pick(srcs, times[r]))
            r += 1
        while lns and lns[0][0] <= t:
            tt, lr = lns.pop(0)
            ln_chunk(nxt_row0, lr, lnr, pick128(srcs, tt))
        if nxt_row0 is not None and not cfg['early']:
            layernorm(nxt_row0, nxt_tm)
        if first:
            dma('wd').wait()
        dn = jnp.dot(get(h_ref, tm), wd[...], preferred_element_type=f32)
        if first:
            dma('wo').wait()
            permute_o()
            x_copy(1).wait()
        per = 11 * tm / 4
        dsrcs = [(t + per * (ct + 0.7) + 0.3 * per * rr / tm, dn[rr + 24:rr + 32, ct * 128:(ct + 1) * 128])
                 for ct in range(4) for rr in range(0, tm - 31, 32)]
        while r < nr:
            while lns and lns[0][0] <= times[r]:
                tt, lr = lns.pop(0)
                ln_chunk(nxt_row0, lr, lnr, pick(dsrcs, tt))
            att_chunk(r * rc, first, pick(dsrcs, times[r]))
            r += 1
        for tt, lr in lns:
            ln_chunk(nxt_row0, lr, lnr, pick(dsrcs, tt))
        halo(tm)
        acc = xb[pl.ds(row0, tm), :].astype(f32) + dn
        acc = acc + jnp.dot(get(o_ref, tm), get(wop), preferred_element_type=f32)
        for tt in range(osplit):
            ob[pl.ds(row0, tm), pl.ds(tt * ow, ow)] = acc[:, tt * ow:(tt + 1) * ow].astype(bf16)
            o_copy(i, tt, row0, tm).start()

    z = jnp.zeros((HALO, 128), f32)
    for j in range(4):
        k_ref[j, pl.ds(0, HALO), :] = z
        v_ref[j, pl.ds(0, HALO), :] = z
    order0 = cfg['order0']
    for name in names:
        if name[0] == 'x' and name != 'x0' and cfg['xloop']:
            continue
        dma(name).start()
    if cfg['xloop']:
        @pl.loop(1, nblk)
        def _(i):
            x_copy_dyn(i).start()
    for waits, starts, steps in order0:
        with jax.named_scope('wait_' + '_'.join(waits)) if cfg['scopes'] else contextless():
            for name in waits:
                dma(name).wait()
            for name in starts:
                dma(name).start()
        for step in steps:
            if step[0] == 'g':
                gate_up(int(step[1:]), tm0, first=True)
            elif step[:2] == 'pq':
                permute_qkv(int(step[2:]))
            elif step == 'po':
                permute_o()
            elif step == 'qkv':
                qkv(tm0)
            elif step[:2] == 'ln':
                layernorm(0, tm0)
            elif step[:5] == 'tail_':
                if cfg['early']:
                    xnb[pl.ds(0, tm0 // 2), :] = xn_ref[pl.ds(0, tm0 // 2), :]
                tail([int(ch) for ch in step[5:]], True, cfg['pace0'][0], cfg['pace0'][1], 0, 0, tm0, tm0, tm1,
                     xnb if cfg['early'] else xn_ref)

    def body(i):
        row0 = pl.multiple_of(tm0 + (i - 1) * tm1, 16)
        nxt = pl.multiple_of(tm0 + (jnp.minimum(i + 1, nblk - 1) - 1) * tm1, 16)
        if cfg['early']:
            xnb[pl.ds(0, tm1 // 2), :] = xn_ref[pl.ds(0, tm1 // 2), :]
            qkv(tm1)
            tail(list(range(len(chunks))), False, cfg['pace'][0], cfg['pace'][1], i, row0, tm1, nxt, tm1, xnb)
        else:
            qkv(tm1)
            tail(list(range(len(chunks))), False, cfg['pace'][0], cfg['pace'][1], i, row0, tm1, nxt, tm1, xn_ref)

    pl.loop(1, nblk)(body)
    with jax.named_scope('wait_out') if cfg['scopes'] else contextless():
        for i in range(nblk):
            r0, n = blk(i)
            for t in range(osplit):
                o_copy(i, t, r0, n).wait()


class contextless:
    def __enter__(self):
        return self

    def __exit__(self, *a):
        return False


def make(tm0=512, tm1=512, rc=8, nc=256, order0=None, unroll=False, packed=True, osplit=4, scopes=False,
         pace=(0, 10500), pace0=(0, 7000), early_x=False, nosem=True, lnp=(300, 10000), lnp0=(6500, 10200), lnr=32, early=True, flags=None, variant='a', xloop=True, mark=192, ln0r=64):
    nch = -(-DF // nc)
    nb = 1 + (S - tm0) // tm1
    tm = max(tm0, tm1)
    xs = ['x%d' % i for i in range(2, nb)]
    if order0 is None:
        pre = [(['x0'], [], ['ln0']),
               ([], [], ['g0']),
               ([], [], ['g1']), (['wq0'], [], ['pq0']),
               ([], [], ['g2']), (['wq1'], [], ['pq1']), (['wq2'], [], ['pq2']),
               ([], [], ['qkv'])]
        if variant == 'a':
            order0 = pre + [([], [], ['tail_345']), (xs, [], [])]
        else:
            order0 = pre + [([], [], ['g3']), ([], [], ['tail_45']), (xs, [], [])]
    names = 'x0 g0 u0 g1 u1 wq0 g2 u2 wq1 wq2 g3 u3 g4 u4 g5 u5 wd wo x1'.split() + xs
    cfg = dict(mark=mark, ln0r=ln0r, names=names, xloop=xloop, tm0=tm0, tm1=tm1, rc=rc, nc=nc, order0=order0, unroll=unroll, packed=packed, osplit=osplit, scopes=scopes,
               pace=pace, pace0=pace0, lnp=lnp, lnp0=lnp0, lnr=lnr, early=early)

    @jax.jit
    def f(A_x, A_wqkv, A_wo, B_x, B_w_gate, B_w_up, B_w_down):
        x2 = A_x.reshape(S, D)
        hbm = pl.BlockSpec(memory_space=pltpu.HBM)
        nblk = nb
        act = (lambda r, c: pltpu.VMEM((r // 2, c), u32)) if packed else (lambda r, c: pltpu.VMEM((r, c), bf16))
        out = pl.pallas_call(
            functools.partial(_kernel, cfg=cfg),
            in_specs=[hbm] * 6,
            out_specs=hbm,
            out_shape=jax.ShapeDtypeStruct((S, D), bf16),
            scratch_shapes=[
                pltpu.VMEM((S, D), bf16), pltpu.VMEM((S, D), bf16),
                pltpu.VMEM((3, D, D), bf16), act(D, 3 * D),
                pltpu.VMEM((D, D), bf16), pltpu.VMEM((4, D, 128), f32), act(D, D),
                pltpu.VMEM((2, DF + 16, D), bf16), pltpu.VMEM((DF, D), bf16),
                act(tm, D), act(tm, D),
                pltpu.VMEM((4, tm, 128), f32),
                pltpu.VMEM((4, tm + HALO, 128), f32),
                pltpu.VMEM((4, tm + HALO, 128), f32),
                act(tm, D),
                act(tm, DF),
                pltpu.SemaphoreType.DMA((len(names),)), pltpu.SemaphoreType.DMA((nblk, osplit)),
            ],
            compiler_params=pltpu.CompilerParams(vmem_limit_bytes=100 * 1024 * 1024, disable_semaphore_checks=nosem, flags=flags if flags is not None else {'XLA_TPU_RESCHEDULE_DMA_DONES': True}),
            name="fused_kernel",
        )(x2, A_wqkv, A_wo, B_w_gate.T, B_w_up.T, B_w_down)
        return out.reshape(1, S, D)
    return f


_impl = make(**{'mark':128})


@jax.jit
def pallas_parallel_sum__sliding_local_dilated__glu_gated_geglu__prompt_kernel(
    A_x: jax.Array,
    A_wqkv: jax.Array,
    A_wo: jax.Array,
    B_x: jax.Array,
    B_w_gate: jax.Array,
    B_w_up: jax.Array,
    B_w_down: jax.Array,
):
    return _impl(A_x, A_wqkv, A_wo, B_x, B_w_gate, B_w_up, B_w_down)
```

```python
import functools

import jax
import jax.numpy as jnp
import jax.experimental.pallas as pl
import jax.experimental.pallas.tpu as pltpu

S, D, H, DH, WIN, DIL, DF = 2048, 512, 32, 16, 8, 2, 1376
TM = 512
NBLK = S // TM
HALO = 16
NC = 256
CHUNKS = [(n0, min(NC, DF - n0)) for n0 in range(0, DF, NC)]
RC = 8
LNR = 32
OW = 128
NOUT = D // OW
LOG2E = 1.4426950408889634
NT = (((1,), (1,)), ((), ()))
f32, bf16, u32 = jnp.float32, jnp.bfloat16, jnp.uint32

DMA_ORDER = ('x0 g0 u0 g1 u1 wq0 g2 u2 wq1 wq2 g3 u3 g4 u4 g5 u5 wd wo'.split()
             + ['x%d' % i for i in range(1, NBLK)])

ATT_PACE_FIRST, LN_PACE_FIRST = (0, 7000), (6500, 10200)
ATT_PACE, LN_PACE = (0, 10500), (300, 10000)


def _gelu(x):
    c = 0.7978845608028654
    return 0.5 * x * (1.0 + jnp.tanh(c * (x + 0.044715 * (x * x * x))))


def _zero_word(v):
    return (pltpu.bitcast(v, u32) >> 31) >> 1


def _kernel(x_hbm, wqkv_hbm, wo_hbm, wg_hbm, wu_hbm, wd_hbm, out_hbm,
            xb, ob, wqkv, wqkvp, wo, wo32, wop, wgu, wd,
            xn, xnb, q_ref, k_ref, v_ref, o_ref, h_ref, sem_in, sem_out):

    def dma(name):
        sem = sem_in.at[DMA_ORDER.index(name)]
        if name[0] == 'x':
            rows = pl.ds(int(name[1:]) * TM, TM)
            return pltpu.make_async_copy(x_hbm.at[rows, :], xb.at[rows, :], sem)
        if name[0] in 'gu':
            n0, nn = CHUNKS[int(name[1:])]
            src = wg_hbm if name[0] == 'g' else wu_hbm
            return pltpu.make_async_copy(src.at[pl.ds(n0, nn), :],
                                         wgu.at['gu'.index(name[0]), pl.ds(n0, nn), :], sem)
        if name[:2] == 'wq':
            m = int(name[2:])
            return pltpu.make_async_copy(wqkv_hbm.at[:, pl.ds(m * D, D)], wqkv.at[m], sem)
        if name == 'wo':
            return pltpu.make_async_copy(wo_hbm, wo, sem)
        return pltpu.make_async_copy(wd_hbm, wd, sem)

    def out_dma(i, t):
        sl = (pl.ds(pl.multiple_of(i * TM, TM), TM), pl.ds(t * OW, OW))
        return pltpu.make_async_copy(ob.at[sl], out_hbm.at[sl], sem_out.at[i, t])

    def put(ref, r0, c0, val):
        ref[pl.ds(r0 // 2, val.shape[0] // 2), pl.ds(c0, val.shape[1])] = pltpu.bitcast(val, u32)

    def get(ref):
        return pltpu.bitcast(ref[...], bf16)

    def ln_chunk(row0, r, n, pace=None, mark=False):
        xv = xb[pl.ds(row0 + r, n), :]
        if pace is not None:
            z = jnp.concatenate([_zero_word(pace)] * (D // 128), axis=1)
            z = jnp.concatenate([z] * (n // 16), axis=0) if n > 16 else z
            xv = pltpu.bitcast(pltpu.bitcast(xv, u32) | z, bf16)
        x = xv.astype(f32)
        xc = x - jnp.mean(x, axis=-1, keepdims=True)
        var = jnp.mean(xc * xc, axis=-1, keepdims=True)
        y = (xc * jax.lax.rsqrt(var + 1e-5)).astype(bf16)
        put(xn, r, 0, y)
        if mark:
            wgu[0, pl.ds(DF, 16), pl.ds(0, 128)] = y[n - 16:n, D - 128:D]

    def permute_qkv(mat):
        lane = jax.lax.broadcasted_iota(jnp.int32, (D // 2, 128), 1)
        grp = (lane % 32) // 8
        tiles = [pltpu.bitcast(wqkv[mat, :, pl.ds(t * 128, 128)], u32) for t in range(4)]
        for j in range(4):
            idx = (lane % 8) * 16 + 4 * j + lane // 32
            res = None
            for t in range(4):
                g = jnp.take_along_axis(tiles[t], idx, axis=1)
                res = g if res is None else jnp.where(grp == t, g, res)
            wqkvp[:, pl.ds(mat * D + j * 128, 128)] = res

    def permute_o():
        for c in range(4):
            wo32[c] = wo[:, pl.ds(c * 128, 128)].astype(f32)
        for c in range(4):
            for d in range(DH):
                put(wop, d * H, c * 128, wo32[c, pl.ds(d, H, stride=DH), :].astype(bf16))

    def qkv():
        def tile(c0):
            w = pltpu.bitcast(wqkvp[:, pl.ds(c0, 128)], bf16)
            return jnp.dot(get(xn), w, preferred_element_type=f32)
        for j in range(4):
            q_ref[j] = tile(j * 128)
        for j in range(4):
            k_ref[j, pl.ds(HALO, TM), :] = tile(D + j * 128)
        for j in range(4):
            v_ref[j, pl.ds(HALO, TM), :] = tile(2 * D + j * 128)

    def gate_up(c, src, first, t0=0.0):
        n0, nn = CHUNKS[c]
        if first:
            dma('g%d' % c).wait()
        g = jax.lax.dot_general(get(src), wgu[0, pl.ds(n0, nn), :], NT, preferred_element_type=f32)
        if first:
            dma('u%d' % c).wait()
        u = jax.lax.dot_general(get(src), wgu[1, pl.ds(n0, nn), :], NT, preferred_element_type=f32)
        put(h_ref, 0, n0, (_gelu(g) * u).astype(bf16))
        marks, t = [], t0
        for val in (g, u):
            for c0 in range(0, nn, 128):
                if nn - c0 >= 128:
                    marks += [(t + r + 32, val[r + 24:r + 32, c0:c0 + 128]) for r in range(0, TM, 32)]
                t += TM
        return marks, t

    def att_chunk(r0, first, pace):
        scale = jnp.full((RC, 128), (DH ** -0.5) * LOG2E, f32)
        scale = pltpu.bitcast(pltpu.bitcast(scale, u32) | _zero_word(pace), f32)
        q = [q_ref[j, pl.ds(r0, RC), :] * scale for j in range(4)]
        logits = []
        for w in range(WIN):
            acc = None
            for j in range(4):
                p = q[j] * k_ref[j, pl.ds(HALO + r0 - DIL * w, RC), :]
                acc = p if acc is None else acc + p
            acc = acc + pltpu.roll(acc, 64, 1)
            acc = acc + pltpu.roll(acc, 32, 1)
            if first and r0 < DIL * w:
                row = r0 + jax.lax.broadcasted_iota(jnp.int32, (RC, 128), 0)
                acc = jnp.where(row >= DIL * w, acc, -1e30)
            logits.append(acc)
        mx = functools.reduce(jnp.maximum, logits)
        es = [jnp.exp2(l - mx) for l in logits]
        rinv = 1.0 / functools.reduce(jnp.add, es)
        outs = []
        for j in range(4):
            o = None
            for w in range(WIN):
                p = es[w] * v_ref[j, pl.ds(HALO + r0 - DIL * w, RC), :]
                o = p if o is None else o + p
            outs.append(o * rinv)
        return outs

    def pick(marks, t):
        return min(marks, key=lambda m: abs(m[0] - t))[1]

    def block_tail(cs, first, i, row0, nxt_row0):
        a_lo, a_hi = ATT_PACE_FIRST if first else ATT_PACE
        l_lo, l_hi = LN_PACE_FIRST if first else LN_PACE
        na, nl = TM // RC, TM // LNR
        todo = sorted([(a_lo + (a_hi - a_lo) * r / (na - 1), 1, r * RC) for r in range(na)]
                      + [(l_lo + (l_hi - l_lo) * r / (nl - 1), 0, r * LNR) for r in range(nl)])
        held = []

        def run(marks, t_end):
            while todo and todo[0][0] <= t_end:
                t, kind, r = todo.pop(0)
                if kind == 0:
                    ln_chunk(nxt_row0, r, LNR, pick(marks, t))
                    continue
                held.append(att_chunk(r, first, pick(marks, t)))
                if len(held) == 16 // RC:
                    for j in range(4):
                        put(o_ref, r + RC - 16, j * 128,
                            jnp.concatenate([h[j] for h in held], axis=0).astype(bf16))
                    held.clear()

        xnb[...] = xn[...]
        marks, t = [], 0.0
        for c in cs:
            m, t = gate_up(c, xnb, first, t)
            marks += m
        run(marks, t)
        if first:
            dma('wd').wait()
        dn = jnp.dot(get(h_ref), wd[...], preferred_element_type=f32)
        if first:
            dma('wo').wait()
            permute_o()
            dma('x1').wait()
        per = 11 * TM / 4
        run([(t + per * (ct + 0.7) + 0.3 * per * r / TM, dn[r + 24:r + 32, ct * 128:(ct + 1) * 128])
             for ct in range(4) for r in range(0, TM, 32)], float('inf'))
        for j in range(4):
            k_ref[j, pl.ds(0, HALO), :] = k_ref[j, pl.ds(TM, HALO), :]
            v_ref[j, pl.ds(0, HALO), :] = v_ref[j, pl.ds(TM, HALO), :]
        acc = xb[pl.ds(row0, TM), :].astype(f32) + dn
        acc = acc + jnp.dot(get(o_ref), get(wop), preferred_element_type=f32)
        for t in range(NOUT):
            ob[pl.ds(row0, TM), pl.ds(t * OW, OW)] = acc[:, t * OW:(t + 1) * OW].astype(bf16)
            out_dma(i, t).start()

    for name in DMA_ORDER[:DMA_ORDER.index('x1')]:
        dma(name).start()

    @pl.loop(1, NBLK)
    def _(i):
        rows = pl.ds(pl.multiple_of(i * TM, TM), TM)
        pltpu.make_async_copy(x_hbm.at[rows, :], xb.at[rows, :],
                              sem_in.at[DMA_ORDER.index('x1') - 1 + i]).start()

    zero = jnp.zeros((HALO, 128), f32)
    for j in range(4):
        k_ref[j, pl.ds(0, HALO), :] = zero
        v_ref[j, pl.ds(0, HALO), :] = zero

    dma('x0').wait()
    for r in range(0, TM, 64):
        ln_chunk(0, r, 64, mark=(r == 128))
    gate_up(0, xn, True)
    gate_up(1, xn, True)
    dma('wq0').wait()
    permute_qkv(0)
    gate_up(2, xn, True)
    for m in (1, 2):
        dma('wq%d' % m).wait()
        permute_qkv(m)
    qkv()
    block_tail(range(3, len(CHUNKS)), True, 0, 0, TM)
    for i in range(2, NBLK):
        dma('x%d' % i).wait()

    @pl.loop(1, NBLK)
    def _(i):
        qkv()
        block_tail(range(len(CHUNKS)), False, i, pl.multiple_of(i * TM, TM),
                   pl.multiple_of(jnp.minimum(i + 1, NBLK - 1) * TM, TM))

    for i in range(NBLK):
        for t in range(NOUT):
            out_dma(i, t).wait()


@jax.jit
def pallas_parallel_sum__sliding_local_dilated__glu_gated_geglu__prompt_kernel(
    A_x: jax.Array,
    A_wqkv: jax.Array,
    A_wo: jax.Array,
    B_x: jax.Array,
    B_w_gate: jax.Array,
    B_w_up: jax.Array,
    B_w_down: jax.Array,
):
    del B_x
    hbm = pl.BlockSpec(memory_space=pltpu.HBM)
    packed = lambda r, c: pltpu.VMEM((r // 2, c), u32)
    out = pl.pallas_call(
        _kernel,
        in_specs=[hbm] * 6,
        out_specs=hbm,
        out_shape=jax.ShapeDtypeStruct((S, D), bf16),
        scratch_shapes=[
            pltpu.VMEM((S, D), bf16),
            pltpu.VMEM((S, D), bf16),
            pltpu.VMEM((3, D, D), bf16),
            packed(D, 3 * D),
            pltpu.VMEM((D, D), bf16),
            pltpu.VMEM((4, D, 128), f32),
            packed(D, D),
            pltpu.VMEM((2, DF + 16, D), bf16),
            pltpu.VMEM((DF, D), bf16),
            packed(TM, D),
            packed(TM, D),
            pltpu.VMEM((4, TM, 128), f32),
            pltpu.VMEM((4, TM + HALO, 128), f32),
            pltpu.VMEM((4, TM + HALO, 128), f32),
            packed(TM, D),
            packed(TM, DF),
            pltpu.SemaphoreType.DMA((len(DMA_ORDER),)),
            pltpu.SemaphoreType.DMA((NBLK, NOUT)),
        ],
        compiler_params=pltpu.CompilerParams(
            vmem_limit_bytes=100 * 1024 * 1024,
            disable_semaphore_checks=True,
            flags={'XLA_TPU_RESCHEDULE_DMA_DONES': True},
        ),
        name="fused_kernel",
    )(A_x.reshape(S, D), A_wqkv, A_wo, B_w_gate.T, B_w_up.T, B_w_down)
    return out.reshape(1, S, D)
```
